```python
import os as _os
_os.environ.setdefault("JAX_PLATFORMS", "cpu")
import jax
import jax.numpy as jnp

def _softmax(x, axis=-1):
    return jax.nn.softmax(x, axis=axis)
def _gelu(x):
    return jax.nn.gelu(x, approximate=True)
def _silu(x):
    return jax.nn.silu(x)
def _sigmoid(x):
    return jax.nn.sigmoid(x)
def _layernorm(x, axis=-1, eps=1e-5):
    m = jnp.mean(x, axis=axis, keepdims=True)
    v = jnp.var(x, axis=axis, keepdims=True)
    return (x - m) / jnp.sqrt(v + eps)
def _scatter_add(tgt, idx, src, axis=0):
    return tgt.at[idx].add(src)
def _segment_sum(src, seg, n):
    return jax.ops.segment_sum(src, seg, n)
class _Rng:
    def __init__(self, key):
        self._k = key
    def _next(self):
        self._k, sub = jax.random.split(self._k)
        return sub
    def normal(self, shape):
        return jax.random.normal(self._next(), shape, dtype=jnp.bfloat16)
    def randint(self, lo, hi, shape):
        return jax.random.randint(self._next(), shape, lo, hi, dtype=jnp.int32)
    def uniform(self, shape, lo=0.0, hi=1.0):
        return jax.random.uniform(self._next(), shape, jnp.bfloat16, lo, hi)
    def permutation(self, n):
        return jax.random.permutation(self._next(), n)


kernel_name = 'standalone__geglu_ffn__prompt'

def setup_inputs():
    _rng = _Rng(jax.random.key(int.from_bytes(__import__("os").urandom(4), "little")))
    _w = (lambda a: (lambda t: t.astype(jnp.bfloat16) if jnp.issubdtype(t.dtype, jnp.floating) else t)(jnp.asarray(a)))
    B, S, D, F = 1, 2048, 576, 4608
    return {
        "x": _w((lambda *s: _rng.normal(s) * 0.05)(B, S, D)),
        "w_gate": _w((lambda *s: _rng.normal(s) * 0.05)(D, F)),
        "w_up": _w((lambda *s: _rng.normal(s) * 0.05)(D, F)),
        "w_down": _w((lambda *s: _rng.normal(s) * 0.05)(F, D)),
    }

def reference(x, w_gate, w_up, w_down):
    return (_gelu(x @ w_gate) * (x @ w_up)) @ w_down
```

```python
import jax
import jax.numpy as jnp
import numpy as np
from jax import lax
import jax.experimental.pallas as pl
import jax.experimental.pallas.tpu as pltpu

_C1 = float(np.sqrt(2.0 / np.pi))
_C2 = float(np.sqrt(2.0 / np.pi) * 0.044715)
_PAIR_RATIO = 3.0


def _geglu(g, u):
    t = jnp.tanh(g * (_C1 + _C2 * (g * g)))
    hg = (0.5 * g) * u
    return hg + hg * t


def _dot(a, b, ca=1, cb=0):
    return lax.dot_general(a, b, (((ca,), (cb,)), ((), ())), preferred_element_type=jnp.float32)


@jax.jit
def pallas_standalone__geglu_ffn__prompt_kernel(
    x: jax.Array,
    w_gate: jax.Array,
    w_up: jax.Array,
    w_down: jax.Array,
):
    bf16, f32 = jnp.bfloat16, jnp.float32
    B, S0, D = x.shape
    S, F = B * S0, w_gate.shape[1]
    c, tp, tn, c0 = 512, 512, 128, 256
    nc, npc, hp, H = F // c, S // tp, tp // 2, S // 2
    KM = (D // 128) * 128
    T = D - KM
    assert T == 64 and F % c == 0 and S % tp == 0 and npc >= 4 and nc >= 3

    def kernel(xT_h, wg_h, wu_h, wdT_h, o_h, xT_v, wg_v, wu_v, wd_v, x1, x2, xq, h1, h2, acc, o_v, flag, sem):
        semA, semB = sem.at[0], sem.at[1]

        def cx(p, s):
            return pltpu.make_async_copy(xT_h.at[:, pl.ds(p * tp, tp)], xT_v.at[p], s)

        def cw(src, dst, j, s, lo=0, n=c):
            return pltpu.make_async_copy(src.at[:, pl.ds(j * c + lo, n)], dst.at[j, :, pl.ds(lo, n)], s)

        def grp(j, s):
            return [cw(wdT_h, wd_v, j - 1, s), cw(wg_h, wg_v, j, s), cw(wu_h, wu_v, j, s)]

        first = [cx(0, semA), cw(wg_h, wg_v, 0, semA, 0, c0), cw(wu_h, wu_v, 0, semA, 0, c0)]
        second = [cw(wg_h, wg_v, 0, semB, c0, c - c0), cw(wu_h, wu_v, 0, semB, c0, c - c0), cx(1, semB)]
        third = [cx(p, semA) for p in range(2, npc)]
        fourth = grp(1, semB)
        rest = [cp for j in range(2, nc) for cp in grp(j, semA)] + [cw(wdT_h, wd_v, nc - 1, semA)]

        def start(cps, priority=1):
            for cp in cps:
                cp.start(priority=priority)

        def wait(cps):
            for cp in cps:
                cp.wait()

        def prep(p):
            a, b = xT_v[p, :, 0:hp], xT_v[p, :, hp:tp]
            r = pl.ds(p * hp, hp)
            xq[r, :] = jnp.concatenate([a[0:T], b[KM:D]], axis=0).T
            a_lo, a_hi, b_lo, b_hi = (t.astype(f32) for t in (a[0:T], a[KM:D], b[0:T], b[KM:D]))
            x1[r, :] = jnp.concatenate([a[T:KM], (a_hi - b_hi).astype(bf16)], axis=0).T
            x2[r, :] = jnp.concatenate([(b_lo - a_lo).astype(bf16), b[T:KM]], axis=0).T
            n = [jnp.sum(jnp.abs(t), axis=0, keepdims=True) for t in (a_lo, a_hi, b_lo, b_hi)]
            ok = (n[3] <= _PAIR_RATIO * n[1]) & (n[0] <= _PAIR_RATIO * n[2]) & (n[0] + n[1] + n[2] + n[3] <= 1e37)
            return jnp.where(ok, 0.0, 1.0)

        def proj(w_v, j, rows, cols):
            q = _dot(xq[rows, :], jnp.concatenate([w_v[j, 0:T, cols], w_v[j, KM:D, cols]], axis=0))
            return _dot(x1[rows, :], w_v[j, T:D, cols]) + q, _dot(x2[rows, :], w_v[j, 0:KM, cols]) + q

        def gate_up(j, r0, nr, lo=0, n=c):
            rows, cols = pl.ds(r0, nr), pl.ds(lo, n)
            g1, g2 = proj(wg_v, j, rows, cols)
            u1, u2 = proj(wu_v, j, rows, cols)
            h1[rows, cols] = _geglu(g1, u1).astype(bf16)
            h2[rows, cols] = _geglu(g2, u2).astype(bf16)

        def out_copy(k, tok, r0=0, nr=D):
            return pltpu.make_async_copy(o_v.at[k, pl.ds(r0, nr)], o_h.at[pl.ds(r0, nr), pl.ds(tok, tn)], semB)

        def ramp():
            start(first, 0)
            start(second)
            acc[...] = jnp.zeros_like(acc)
            wait(first)
            start(third)
            bad = prep(0)
            gate_up(0, 0, hp, 0, c0)
            wait(second)
            start(fourth)
            gate_up(0, 0, hp, c0, c - c0)
            bad += prep(1)
            gate_up(0, hp, hp, 0, c0)
            wait(third)
            start(rest)
            gate_up(0, hp, hp, c0, c - c0)
            for p in range(2, npc):
                bad += prep(p)
            safe = jnp.max(bad) == 0.0
            gate_up(0, 2 * hp, H - 2 * hp)
            wait(fourth)
            return safe

        def shared():
            def body(j, carry):
                w = wd_v[j - 1]
                acc[:, 0:H] += _dot(w, h1[...], 1, 1)
                acc[:, H:S] += _dot(w, h2[...], 1, 1)
                gate_up(j, 0, H)
                pl.when(j == 1)(lambda: wait(rest))
                return carry

            lax.fori_loop(1, nc, body, 0)
            k = 0
            for s, hh in enumerate((h1, h2)):
                for r0 in range(0, H, tn):
                    tok = (r0 // hp) * tp + s * hp + r0 % hp
                    q0 = 0
                    for nr in ((D // 2, D // 3, D // 6) if k == S // tn - 1 else (D,)):
                        o = acc[q0:q0 + nr, k * tn:(k + 1) * tn] + _dot(wd_v[nc - 1, q0:q0 + nr], hh[r0:r0 + tn, :], 1, 1)
                        o_v[k, q0:q0 + nr] = o.astype(bf16)
                        out_copy(k, tok, q0, nr).start()
                        q0 += nr
                    k += 1

        def plain():
            def chunk(j, carry):
                pl.when(j == 1)(lambda: wait(rest))

                def tile(t, carry):
                    xt = xT_v[t // 2, :, pl.ds(pl.multiple_of((t % 2) * hp, hp), hp)]
                    h = _geglu(_dot(wg_v[j], xt, 0, 0), _dot(wu_v[j], xt, 0, 0)).astype(bf16)
                    acc[:, pl.ds(pl.multiple_of(t * hp, hp), hp)] += _dot(wd_v[j], h)
                    return carry

                return lax.fori_loop(0, S // hp, tile, carry)

            lax.fori_loop(0, nc, chunk, 0)

            def put(k, carry):
                tok = pl.multiple_of(k * tn, tn)
                o_v[k] = acc[:, pl.ds(tok, tn)].astype(bf16)
                out_copy(k, tok).start()
                return carry

            lax.fori_loop(0, S // tn, put, 0)

        def attempt(state):
            @pl.when(state == 1)
            def _():
                plain()
                flag[0] = 2

            @pl.when(state == 0)
            def _():
                safe = ramp()
                flag[0] = jnp.where(safe, 2, 1)
                pl.when(safe)(shared)

            return flag[0]

        flag[0] = 0
        lax.while_loop(lambda state: state < 2, attempt, 0)
        pltpu.make_async_copy(o_v, o_v, semB).wait()

    hbm = pl.BlockSpec(memory_space=pl.ANY)
    out_t = pl.pallas_call(
        kernel,
        in_specs=[hbm] * 4,
        out_specs=hbm,
        out_shape=jax.ShapeDtypeStruct((D, S), x.dtype),
        scratch_shapes=(
            [pltpu.VMEM((npc, D, tp), bf16)]
            + [pltpu.VMEM((nc, D, c), bf16)] * 3
            + [pltpu.VMEM((H, KM), bf16)] * 2
            + [pltpu.VMEM((H, 2 * T), bf16)]
            + [pltpu.VMEM((H, c), bf16)] * 2
            + [pltpu.VMEM((D, S), f32), pltpu.VMEM((S // tn, D, tn), bf16)]
            + [pltpu.SMEM((1,), jnp.int32), pltpu.SemaphoreType.DMA((2,))]
        ),
        compiler_params=pltpu.CompilerParams(vmem_limit_bytes=100 * 2**20),
    )(x.reshape(S, D).T, w_gate, w_up, w_down.T)
    return out_t.T.reshape(B, S0, D)
```

```python
import jax
import jax.numpy as jnp
import numpy as np
from jax import lax
import jax.experimental.pallas as pl
import jax.experimental.pallas.tpu as pltpu

_GELU_C1 = float(np.sqrt(2.0 / np.pi))
_GELU_C3 = float(np.sqrt(2.0 / np.pi) * 0.044715)
_PAIR_RATIO = 3.0

_HALF = 128
_PIECE = 2 * _HALF
_CHUNK = 512
_LEAD = 6
_STEP = 11


def _geglu(g, u):
    t = jnp.tanh(g * (_GELU_C1 + _GELU_C3 * (g * g)))
    half_gu = (0.5 * g) * u
    return (half_gu + half_gu * t).astype(jnp.bfloat16)


def _dot(a, b, ca=1, cb=0):
    dims = (((ca,), (cb,)), ((), ()))
    return lax.dot_general(a, b, dims, preferred_element_type=jnp.float32)


def _block(i, size, count=1):
    start = i * size if isinstance(i, int) else pl.multiple_of(i * size, size)
    return pl.ds(start, count * size)


@jax.jit
def pallas_standalone__geglu_ffn__prompt_kernel(
    x: jax.Array,
    w_gate: jax.Array,
    w_up: jax.Array,
    w_down: jax.Array,
):
    bf16, f32 = jnp.bfloat16, jnp.float32
    D, F = w_gate.shape
    S = x.size // D
    n_piece, n_chunk = S // _PIECE, F // _CHUNK
    n_iter = (n_piece * n_chunk - _LEAD) // _STEP
    LO, HI = D - 128, D - 64
    K0, C0, C1 = 256, 256, 384
    assert D % 128 == 64 and LO > K0
    assert S == n_piece * _PIECE and F == n_chunk * _CHUNK
    assert n_iter * _STEP + _LEAD == n_piece * n_chunk
    assert 4 < _LEAD <= n_piece and _LEAD < _STEP <= 2 * min(_LEAD, n_piece)

    def kernel(xt_hbm, wg_hbm, wu_hbm, wdt_hbm, out_hbm,
               xt, wg, wu, wdt, xa, xb, xq, part, h, acc, out, state, sems):
        def load_x(s, p0, p1, k0=0, k1=D):
            at = (pl.ds(k0, k1 - k0), _block(p0, _PIECE, p1 - p0))
            return [pltpu.make_async_copy(xt_hbm.at[at], xt.at[at], sems.at[s])]

        def load_w(src, dst, s, j, c0=0, c1=_CHUNK, k0=0, k1=D):
            rows = pl.ds(k0, k1 - k0)
            return pltpu.make_async_copy(
                src.at[rows, pl.ds(j * _CHUNK + c0, c1 - c0)],
                dst.at[j, rows, pl.ds(c0, c1 - c0)], sems.at[s])

        def load_gu(*args):
            return [load_w(wg_hbm, wg, *args), load_w(wu_hbm, wu, *args)]

        def load_d(*args):
            return [load_w(wdt_hbm, wdt, *args)]

        loads = [
            load_x(0, 0, 2, 0, K0) + load_gu(0, 0, 0, C0, 0, K0),
            load_x(1, 0, 2, K0, D) + load_gu(1, 0, 0, C0, K0, D),
            load_gu(0, 0, C0, C1) + load_x(0, 2, 3),
            load_gu(1, 0, C1, _CHUNK) + load_x(1, 3, n_piece),
            load_gu(0, 1) + load_gu(0, 2) + load_d(0, 0) + load_d(0, 1),
            sum((load_gu(1, j) for j in range(3, n_chunk)), [])
            + sum((load_d(1, j) for j in range(2, n_chunk)), []),
        ]

        def start(group):
            for copy in loads[group]:
                copy.start()

        def wait(group):
            for copy in loads[group]:
                copy.wait()

        def write_out(blk, r0=0, n=D):
            pltpu.make_async_copy(
                out.at[blk, pl.ds(r0, n)],
                out_hbm.at[pl.ds(r0, n), _block(blk, _HALF)], sems.at[0]).start()

        def pair_up(p, k0=0):
            rows, ta, tb = _block(p, _HALF), _block(2 * p, _HALF), _block(2 * p + 1, _HALF)
            a_lo, a_hi, b_lo, b_hi = xt[LO:HI, ta], xt[HI:D, ta], xt[LO:HI, tb], xt[HI:D, tb]
            xq[rows, :] = jnp.concatenate([a_lo, b_hi], axis=0).T
            a_lo, a_hi, b_lo, b_hi = (v.astype(f32) for v in (a_lo, a_hi, b_lo, b_hi))
            xa[rows, k0:HI] = jnp.concatenate([xt[k0:LO, ta], (a_hi - b_hi).astype(bf16)], axis=0).T
            xb[rows, k0:HI] = jnp.concatenate([xt[k0:LO, tb], (b_lo - a_lo).astype(bf16)], axis=0).T
            a_lo, a_hi, b_lo, b_hi = (
                jnp.sum(jnp.abs(v), axis=0, keepdims=True) for v in (a_lo, a_hi, b_lo, b_hi))
            safe = ((b_hi <= _PAIR_RATIO * a_hi) & (a_lo <= _PAIR_RATIO * b_lo)
                    & (a_lo + a_hi + b_lo + b_hi <= 1e37))
            return jnp.where(safe, 0.0, 1.0)

        def project(w, j, rows, cols, k0):
            q = _dot(xq[rows, :], w[j, LO:D, cols])
            w_a = jnp.concatenate([w[j, k0:LO, cols], w[j, HI:D, cols]], axis=0)
            return (_dot(xa[rows, k0:HI], w_a) + q,
                    _dot(xb[rows, k0:HI], w[j, k0:HI, cols]) + q)

        def gate_up(j, p, n, slot, c0=0, c1=_CHUNK, k0=0):
            rows, cols = _block(p, _HALF, n), pl.ds(c0, c1 - c0)
            ga, gb = project(wg, j, rows, cols, k0)
            ua, ub = project(wu, j, rows, cols, k0)
            if k0:
                ga, gb, ua, ub = ga + part[0], gb + part[1], ua + part[2], ub + part[3]
            h[slot:slot + n, :_HALF, cols] = _geglu(ga, ua).reshape(n, _HALF, c1 - c0)
            h[slot:slot + n, _HALF:, cols] = _geglu(gb, ub).reshape(n, _HALF, c1 - c0)

        def ramp():
            start(0)
            start(1)

            @pl.loop(0, n_piece)
            def _(p):
                acc[p] = jnp.zeros((D, _PIECE), f32)

            wait(0)
            start(2)
            for p in range(2):
                xa[_block(p, _HALF), :K0] = xt[:K0, _block(2 * p, _HALF)].T
                xb[_block(p, _HALF), :K0] = xt[:K0, _block(2 * p + 1, _HALF)].T
            for i, (w, lhs) in enumerate(((wg, xa), (wg, xb), (wu, xa), (wu, xb))):
                part[i] = _dot(lhs[:2 * _HALF, :K0], w[0, :K0, :C0])
            wait(1)
            start(3)
            unsafe = pair_up(0, K0) + pair_up(1, K0)
            gate_up(0, 0, 2, 0, 0, C0, K0)
            wait(2)
            start(4)
            gate_up(0, 0, 2, 0, C0, C1)
            unsafe += pair_up(2)
            gate_up(0, 2, 1, 2, 0, C1)
            wait(3)
            gate_up(0, 0, 3, 0, C1, _CHUNK)
            unsafe += pair_up(3)
            start(5)
            gate_up(0, 3, 1, 3)
            unsafe += sum(pair_up(p) for p in range(4, n_piece))
            safe = jnp.max(unsafe) == 0.0
            gate_up(0, 4, _LEAD - 4, 4)
            wait(4)
            return safe

        def paired():
            @pl.loop(0, n_iter)
            def _(i):
                def up(t, slot):
                    unit = i * _STEP + _LEAD + t
                    gate_up(unit // n_piece, unit % n_piece, 1, slot)

                def down(t):
                    unit = i * _STEP + t
                    acc[unit % n_piece] += _dot(wdt[unit // n_piece], h[t], 1, 1)

                for t in range(_STEP - _LEAD):
                    up(t, _LEAD + t)
                for t in range(_LEAD):
                    down(t)
                for t in range(_STEP - _LEAD, _STEP):
                    up(t, t - (_STEP - _LEAD))
                for t in range(_LEAD, _STEP):
                    down(t)
                pl.when(i == 0)(lambda: wait(5))

            for blk in range(2 * n_piece):
                p, cols = blk // 2, _block(blk % 2, _HALF)
                slot = p - (n_piece - _LEAD)
                r0 = 0
                for n in ((D // 2, D // 3, D // 6) if blk == 2 * n_piece - 1 else (D,)):
                    rows = pl.ds(r0, n)
                    o = acc[p, rows, cols]
                    if slot >= 0:
                        o = o + _dot(wdt[n_chunk - 1, rows], h[slot, cols, :], 1, 1)
                    out[blk, rows] = o.astype(out.dtype)
                    write_out(blk, r0, n)
                    r0 += n

        def plain():
            @pl.loop(0, n_chunk)
            def _(j):
                pl.when(j == 2)(lambda: wait(5))

                @pl.loop(0, n_piece)
                def _(p):
                    xp = xt[:, _block(p, _PIECE)]
                    acc[p] += _dot(wdt[j], _geglu(_dot(wg[j], xp, 0, 0), _dot(wu[j], xp, 0, 0)))

            @pl.loop(0, 2 * n_piece)
            def _(blk):
                out[blk] = acc[blk // 2, :, _block(blk % 2, _HALF)].astype(out.dtype)
                write_out(blk)

        def attempt(current):
            @pl.when(current == 1)
            def _():
                plain()
                state[0] = 2

            @pl.when(current == 0)
            def _():
                safe = ramp()
                state[0] = jnp.where(safe, 2, 1)
                pl.when(safe)(paired)

            return state[0]

        lax.while_loop(lambda current: current < 2, attempt, 0)
        pltpu.make_async_copy(out, out, sems.at[0]).wait()

    in_hbm = pl.BlockSpec(memory_space=pl.ANY)
    out_t = pl.pallas_call(
        kernel,
        in_specs=[in_hbm] * 4,
        out_specs=in_hbm,
        out_shape=jax.ShapeDtypeStruct((D, S), x.dtype),
        scratch_shapes=[
            pltpu.VMEM((D, S), bf16),
            pltpu.VMEM((n_chunk, D, _CHUNK), bf16),
            pltpu.VMEM((n_chunk, D, _CHUNK), bf16),
            pltpu.VMEM((n_chunk, D, _CHUNK), bf16),
            pltpu.VMEM((S // 2, HI), bf16),
            pltpu.VMEM((S // 2, HI), bf16),
            pltpu.VMEM((S // 2, D - LO), bf16),
            pltpu.VMEM((4, 2 * _HALF, C0), f32),
            pltpu.VMEM((_STEP, _PIECE, _CHUNK), bf16),
            pltpu.VMEM((n_piece, D, _PIECE), f32),
            pltpu.VMEM((2 * n_piece, D, _HALF), x.dtype),
            pltpu.SMEM((1,), jnp.int32),
            pltpu.SemaphoreType.DMA((2,)),
        ],
        compiler_params=pltpu.CompilerParams(vmem_limit_bytes=64 * 2**20),
    )(x.reshape(S, D).T, w_gate, w_up, w_down.T)
    return out_t.T.reshape(x.shape)
```
